```python
import jax
import jax.numpy as jnp

def _softmax(x, axis=-1):
    return jax.nn.softmax(x, axis=axis)
def _gelu(x):
    return jax.nn.gelu(x, approximate=True)
def _silu(x):
    return jax.nn.silu(x)
def _sigmoid(x):
    return jax.nn.sigmoid(x)
def _layernorm(x, axis=-1, eps=1e-5):
    m = jnp.mean(x, axis=axis, keepdims=True)
    v = jnp.var(x, axis=axis, keepdims=True)
    return (x - m) / jnp.sqrt(v + eps)
def _scatter_add(tgt, idx, src, axis=0):
    return tgt.at[idx].add(src)
def _segment_sum(src, seg, n):
    return jax.ops.segment_sum(src, seg, n)
class _Rng:
    def __init__(self, key):
        self._k = key
    def _next(self):
        self._k, sub = jax.random.split(self._k)
        return sub
    def normal(self, shape):
        return jax.random.normal(self._next(), shape, dtype=jnp.bfloat16)
    def randint(self, lo, hi, shape):
        return jax.random.randint(self._next(), shape, lo, hi, dtype=jnp.int32)
    def uniform(self, shape, lo=0.0, hi=1.0):
        return jax.random.uniform(self._next(), shape, jnp.bfloat16, lo, hi)
    def permutation(self, n):
        return jax.random.permutation(self._next(), n)


kernel_name = 'standalone__standard_2d_1d_3d_conv__vision'

def setup_inputs():
    _rng = _Rng(jax.random.key(int.from_bytes(__import__("os").urandom(4), "little")))
    _w = (lambda a: (lambda t: t.astype(jnp.bfloat16) if jnp.issubdtype(t.dtype, jnp.floating) else t)(jnp.asarray(a)))
    H = W = 384
    C = 384
    K = 1
    return {
        "x": _w((lambda *s: _rng.normal(s) * 0.05)(1, H, W, C)),
        "w": _w((lambda *s: _rng.normal(s) * 0.05)(K, K, C, C)),
        "b": _w((lambda *s: _rng.normal(s) * 0.05)(C)),
    }

def reference(x, w, b):
    B, H, W, Cin = x.shape
    K = w.shape[0]
    pl = (K - 1) // 2
    pr = K // 2
    xp = jnp.pad(x, ((0, 0), (pl, pr), (pl, pr), (0, 0)))
    out = sum(
        jnp.einsum('bhwc,cd->bhwd', xp[:, i:i+H, j:j+W, :], w[i, j])
        for i in range(K) for j in range(K)
    )
    return out + b[None, None, None, :]
```

```python
import jax
import jax.numpy as jnp
from jax import lax
import jax.experimental.pallas as pl
import jax.experimental.pallas.tpu as pltpu

A, U, RD, RW, LA = 8, 64, 64, 32, 8


@jax.jit
def pallas_standalone__standard_2d_1d_3d_conv__vision_kernel(
    x: jax.Array,
    w: jax.Array,
    b: jax.Array,
):
    B, H, W, C = x.shape
    D = w.shape[-1]
    assert w.shape[0] == 1 and w.shape[1] == 1 and C == D
    M = B * H * W
    L = M // A
    NU = L // U
    assert NU * U * A == M

    def kernel_function(x_hbm, w_hbm, b_hbm, o_hbm, buf, w_v, b_v, rsem, wsem, csem):
        def rd_start(u):
            off = pl.multiple_of(u * U, U)
            for a in range(A):
                pltpu.make_async_copy(
                    x_hbm.at[pl.ds(a, 1), pl.ds(off, RD)], buf.at[pl.ds(a, 1), pl.ds(off, RD)], rsem.at[u % LA]
                ).start(priority=a % 2)

        def rd_wait(u):
            off = pl.multiple_of(u * U, U)
            pltpu.make_async_copy(x_hbm.at[:, pl.ds(off, U)], buf.at[:, pl.ds(off, U)], rsem.at[u % LA]).wait()

        def wr_start(u):
            for r in range(U // RW):
                off = pl.multiple_of(u * U + r * RW, RW)
                pltpu.make_async_copy(
                    buf.at[:, pl.ds(off, RW)], o_hbm.at[:, pl.ds(off, RW)], wsem.at[u % LA]
                ).start()

        def wr_wait(u):
            off = pl.multiple_of(u * U, U)
            pltpu.make_async_copy(buf.at[:, pl.ds(off, U)], o_hbm.at[:, pl.ds(off, U)], wsem.at[u % LA]).wait()

        def compute(u):
            off = pl.multiple_of(u * U, U)
            xv = buf[:, pl.ds(off, U), :].reshape(A * U, C)
            acc = jnp.dot(xv, w_v[...], preferred_element_type=jnp.float32)
            acc = acc + b_v[...].astype(jnp.float32).reshape(1, D)
            buf[:, pl.ds(off, U), :] = acc.astype(buf.dtype).reshape(A, U, D)

        rd_start(0)
        cw = pltpu.make_async_copy(w_hbm, w_v, csem.at[0])
        cb = pltpu.make_async_copy(b_hbm, b_v, csem.at[1])
        cw.start()
        cb.start()

        def pro(u, _):
            rd_start(u)

        lax.fori_loop(1, LA, pro, None)
        cw.wait()
        cb.wait()

        S = NU - LA

        def step(s, _):
            for k in range(2):
                d = 2 * s + k
                pl.when(d < NU)(lambda: rd_wait(d))
                pl.when(d >= NU)(lambda: wr_wait(d - NU))
            for k in range(2):
                d = 2 * s + k + LA
                pl.when(d < NU)(lambda: rd_start(d))
                pl.when(d >= NU)(lambda: wr_start(d - NU))
            compute(s)

        lax.fori_loop(0, S, step, None)

        def tail(s, _):
            compute(s)
            wr_wait(s - LA)
            wr_start(s)

        lax.fori_loop(S, NU, tail, None)

        def fin(s, _):
            wr_wait(s)

        lax.fori_loop(S, NU, fin, None)

    out = pl.pallas_call(
        kernel_function,
        in_specs=[pl.BlockSpec(memory_space=pl.ANY)] * 3,
        out_specs=pl.BlockSpec(memory_space=pl.ANY),
        out_shape=jax.ShapeDtypeStruct((A, L, D), x.dtype),
        scratch_shapes=[
            pltpu.VMEM((A, L, C), x.dtype),
            pltpu.VMEM((C, D), w.dtype),
            pltpu.VMEM((D,), b.dtype),
            pltpu.SemaphoreType.DMA((LA,)),
            pltpu.SemaphoreType.DMA((LA,)),
            pltpu.SemaphoreType.DMA((2,)),
        ],
        compiler_params=pltpu.CompilerParams(
            vmem_limit_bytes=120 * 1024 * 1024, disable_bounds_checks=True
        ),
    )(x.reshape(A, L, C), w.reshape(C, D), b)
    return out.reshape(B, H, W, D)
```

```python
import jax
import jax.numpy as jnp
from jax import lax
import jax.experimental.pallas as pl
import jax.experimental.pallas.tpu as pltpu

A, U = 8, 64
RA, RD = 2, 32
RW = 32
LA = 12
NSUB = 8


@jax.jit
def pallas_standalone__standard_2d_1d_3d_conv__vision_kernel(
    x: jax.Array,
    w: jax.Array,
    b: jax.Array,
):
    B, H, W, C = x.shape
    D = w.shape[-1]
    assert w.shape[0] == 1 and w.shape[1] == 1
    M = B * H * W
    L = M // A
    NU = L // U
    assert NU * U * A == M
    S1 = (NU - LA) // 2
    S = NU - LA
    NX = NU - S1 + 1
    NY = NU // 2 + 2

    def kernel_function(x_hbm, w_hbm, b_hbm, o_hbm, xb, yb, w_v, b_v, rsem, wsem, csem):
        def slot(u, n):
            return jnp.where(u >= n, u - n, u)

        def rd_list(u):
            out = []
            for r in range(U // RD):
                for a in range(0, A, RA):
                    def go(r=r, a=a, k=len(out)):
                        off = pl.multiple_of(u * U + r * RD, RD)
                        pltpu.make_async_copy(
                            x_hbm.at[pl.ds(a, RA), pl.ds(off, RD)],
                            xb.at[slot(u, NX), pl.ds(a, RA), pl.ds(r * RD, RD)],
                            rsem.at[u % LA],
                        ).start(priority=k % 2)
                    out.append(go)
            return out

        def rd_wait(u):
            pltpu.make_async_copy(x_hbm.at[:, pl.ds(0, U)], xb.at[slot(u, NX)], rsem.at[u % LA]).wait()

        def wr_start(u):
            for r in range(U // RW):
                off = pl.multiple_of(u * U + r * RW, RW)
                pltpu.make_async_copy(
                    yb.at[slot(u, NY), :, pl.ds(r * RW, RW)],
                    o_hbm.at[:, pl.ds(off, RW)],
                    wsem.at[u % LA],
                ).start()

        def wr_wait(u):
            pltpu.make_async_copy(yb.at[slot(u, NY)], o_hbm.at[:, pl.ds(0, U)], wsem.at[u % LA]).wait()

        def compute(u, a, na):
            xv = xb[slot(u, NX), pl.ds(a, na)].reshape(na * U, C)
            acc = jnp.dot(xv, w_v[...], preferred_element_type=jnp.float32)
            acc = acc + b_v[...].astype(jnp.float32).reshape(1, D)
            yb[slot(u, NY), pl.ds(a, na)] = acc.astype(yb.dtype).reshape(na, U, D)

        for f in rd_list(0):
            f()
        cw = pltpu.make_async_copy(w_hbm, w_v, csem.at[0])
        cb = pltpu.make_async_copy(b_hbm, b_v, csem.at[1])
        cw.start()
        cb.start()

        def pro(u, _):
            for f in rd_list(u):
                f()

        lax.fori_loop(1, LA, pro, None)
        cw.wait()
        cb.wait()

        def step_r(s, _):
            rd_wait(2 * s)
            rd_wait(2 * s + 1)
            dmas = rd_list(2 * s + LA) + rd_list(2 * s + 1 + LA)
            per = len(dmas) // NSUB
            na = A // NSUB
            for i in range(NSUB):
                for f in dmas[i * per:(i + 1) * per]:
                    f()
                compute(s, i * na, na)

        lax.fori_loop(0, S1, step_r, None)

        def step_w(s, _):
            for k in range(2):
                d = 2 * s + k
                pl.when(d < NU)(lambda: rd_wait(d))
                pl.when(d >= NU)(lambda: wr_wait(d - NU))
            wr_start(2 * s + LA - NU)
            wr_start(2 * s + 1 + LA - NU)
            compute(s, 0, A)

        lax.fori_loop(S1, S, step_w, None)

        def tail(s, _):
            compute(s, 0, A)
            wr_wait(s - LA)
            wr_start(s)

        lax.fori_loop(S, NU, tail, None)

        def fin(s, _):
            wr_wait(s)

        lax.fori_loop(S, NU, fin, None)

    out = pl.pallas_call(
        kernel_function,
        in_specs=[pl.BlockSpec(memory_space=pl.ANY)] * 3,
        out_specs=pl.BlockSpec(memory_space=pl.ANY),
        out_shape=jax.ShapeDtypeStruct((A, L, D), x.dtype),
        scratch_shapes=[
            pltpu.VMEM((NX, A, U, C), x.dtype),
            pltpu.VMEM((NY, A, U, D), x.dtype),
            pltpu.VMEM((C, D), w.dtype),
            pltpu.VMEM((D,), b.dtype),
            pltpu.SemaphoreType.DMA((LA,)),
            pltpu.SemaphoreType.DMA((LA,)),
            pltpu.SemaphoreType.DMA((2,)),
        ],
        compiler_params=pltpu.CompilerParams(
            vmem_limit_bytes=127 * 1024 * 1024, disable_bounds_checks=True
        ),
    )(x.reshape(A, L, C), w.reshape(C, D), b)
    return out.reshape(B, H, W, D)
```

```python
import jax
import jax.numpy as jnp
from jax import lax
import jax.experimental.pallas as pl
import jax.experimental.pallas.tpu as pltpu

STREAMS = 8
UNIT = 64
SEG = 32
READ_AHEAD = 8
WRITE_LAG = 16


@jax.jit
def pallas_standalone__standard_2d_1d_3d_conv__vision_kernel(
    x: jax.Array,
    w: jax.Array,
    b: jax.Array,
):
    B, H, W, C = x.shape
    D = w.shape[-1]
    assert w.shape[0] == 1 and w.shape[1] == 1
    rows = B * H * W
    slab = rows // STREAMS
    n_units = slab // UNIT
    assert n_units * UNIT * STREAMS == rows and n_units % 2 == 0
    read_steps = (n_units - READ_AHEAD) // 2
    n_rsem = READ_AHEAD // 2
    n_x = n_units - read_steps + 1
    n_y = (n_units + WRITE_LAG + 2 - READ_AHEAD) // 2 + 1
    assert 2 * n_x >= n_units and 2 * n_y >= n_units

    def kernel_function(x_hbm, w_hbm, b_hbm, o_hbm, xb, yb, w_v, b_v, rsem, wsem, csem):
        def slot(u, n):
            return jnp.where(u >= n, u - n, u)

        def read_start(u, seg, stream, queue):
            off = pl.multiple_of(u * UNIT + seg * SEG, SEG)
            pltpu.make_async_copy(
                x_hbm.at[stream, pl.ds(off, SEG)],
                xb.at[slot(u, n_x), stream, pl.ds(seg * SEG, SEG)],
                rsem.at[(u // 2) % n_rsem],
            ).start(priority=queue)

        def reads_of(u):
            return [(u, seg, a) for seg in range(UNIT // SEG) for a in range(STREAMS)]

        def read_wait_pair(p):
            for k in range(2):
                pltpu.make_async_copy(
                    x_hbm.at[:, pl.ds(0, UNIT)], xb.at[slot(2 * p + k, n_x)], rsem.at[p % n_rsem]
                ).wait()

        def write_wait(u):
            pltpu.make_async_copy(
                yb.at[slot(u, n_y)], o_hbm.at[:, pl.ds(0, UNIT)], wsem.at[u % WRITE_LAG]
            ).wait()

        def write_start(u):
            pl.when(u >= WRITE_LAG)(lambda: write_wait(u - WRITE_LAG))
            for seg in range(UNIT // SEG):
                off = pl.multiple_of(u * UNIT + seg * SEG, SEG)
                pltpu.make_async_copy(
                    yb.at[slot(u, n_y), :, pl.ds(seg * SEG, SEG)],
                    o_hbm.at[:, pl.ds(off, SEG)],
                    wsem.at[u % WRITE_LAG],
                ).start()

        def compute(u, a, n):
            xv = xb[slot(u, n_x), pl.ds(a, n)].reshape(n * UNIT, C)
            acc = jnp.dot(xv, w_v[...], preferred_element_type=jnp.float32)
            acc = acc + b_v[...].astype(jnp.float32).reshape(1, D)
            yb[slot(u, n_y), pl.ds(a, n)] = acc.astype(yb.dtype).reshape(n, UNIT, D)

        def prologue_backlog(u, _):
            for r in reads_of(u):
                read_start(*r, queue=1)

        def prologue_rest(u, _):
            for k, r in enumerate(reads_of(u)):
                read_start(*r, queue=k % 2)

        w_copy = pltpu.make_async_copy(w_hbm, w_v, csem.at[0])
        b_copy = pltpu.make_async_copy(b_hbm, b_v, csem.at[1])
        lax.fori_loop(0, READ_AHEAD // 2, prologue_backlog, None)
        w_copy.start()
        b_copy.start()
        lax.fori_loop(READ_AHEAD // 2, READ_AHEAD, prologue_rest, None)
        w_copy.wait()
        b_copy.wait()

        def read_step(s, _):
            read_wait_pair(s)
            reads = reads_of(2 * s + READ_AHEAD) + reads_of(2 * s + 1 + READ_AHEAD)
            per = len(reads) // STREAMS
            for a in range(STREAMS):
                for k in range(a * per, (a + 1) * per):
                    read_start(*reads[k], queue=k % 2)
                compute(s, a, 1)

        lax.fori_loop(0, read_steps, read_step, None)

        def write_step(s, nxt):
            pl.when(s < n_units // 2)(lambda: read_wait_pair(s))
            write_start(nxt)
            two = nxt + 1 < s
            pl.when(two)(lambda: write_start(nxt + 1))
            compute(s, 0, STREAMS)
            return nxt + 1 + two.astype(jnp.int32)

        lax.fori_loop(read_steps, n_units, write_step, jnp.int32(0))
        write_start(n_units - 1)

        def drain(u, _):
            write_wait(u)

        lax.fori_loop(n_units - WRITE_LAG, n_units, drain, None)

    out = pl.pallas_call(
        kernel_function,
        in_specs=[pl.BlockSpec(memory_space=pl.ANY)] * 3,
        out_specs=pl.BlockSpec(memory_space=pl.ANY),
        out_shape=jax.ShapeDtypeStruct((STREAMS, slab, D), x.dtype),
        scratch_shapes=[
            pltpu.VMEM((n_x, STREAMS, UNIT, C), x.dtype),
            pltpu.VMEM((n_y, STREAMS, UNIT, D), x.dtype),
            pltpu.VMEM((C, D), w.dtype),
            pltpu.VMEM((D,), b.dtype),
            pltpu.SemaphoreType.DMA((n_rsem,)),
            pltpu.SemaphoreType.DMA((WRITE_LAG,)),
            pltpu.SemaphoreType.DMA((2,)),
        ],
        compiler_params=pltpu.CompilerParams(
            vmem_limit_bytes=127 * 1024 * 1024,
            disable_bounds_checks=True,
            disable_semaphore_checks=True,
        ),
    )(x.reshape(STREAMS, slab, C), w.reshape(C, D), b)
    return out.reshape(B, H, W, D)
```

```python
import jax
import jax.numpy as jnp
from jax import lax
import jax.experimental.pallas as pl
import jax.experimental.pallas.tpu as pltpu

SLAB = 4096
GROUP = 6
UNIT = 64
READ_SEG = 16
WRITE_SEG = 32
READ_QUEUES = (0, 1, 1)
READ_AHEAD = 4
WRITE_LAG = 16


@jax.jit
def pallas_standalone__standard_2d_1d_3d_conv__vision_kernel(
    x: jax.Array,
    w: jax.Array,
    b: jax.Array,
):
    B, H, W, C = x.shape
    D = w.shape[-1]
    assert w.shape[0] == 1 and w.shape[1] == 1
    rows = B * H * W
    n_slabs = rows // SLAB
    per_group = SLAB // UNIT
    n_units = (n_slabs // GROUP) * per_group
    assert n_slabs * SLAB == rows and n_slabs % (2 * GROUP) == 0
    n_pairs = n_units // 2
    read_steps = n_pairs - READ_AHEAD
    n_x = n_units - read_steps + 1
    n_y = (n_units + WRITE_LAG + 2 - 2 * READ_AHEAD) // 2 + 1
    assert 2 * n_x >= n_units and 2 * n_y >= n_units

    def kernel_function(x_hbm, w_hbm, b_hbm, o_hbm, xb, yb, w_v, b_v, rsem, wsem, csem):
        def slot(u, n):
            return jnp.where(u >= n, u - n, u)

        def window(ref, u, slab, n, row, n_rows):
            off = pl.multiple_of((u % per_group) * UNIT + row, 16)
            return ref.at[pl.ds((u // per_group) * GROUP + slab, n), pl.ds(off, n_rows)]

        def pair_units(p):
            u = (p // per_group) * (2 * per_group) + p % per_group
            return u, u + per_group

        pair_reads = [
            (half, slab, row)
            for row in range(0, UNIT, READ_SEG)
            for half in range(2)
            for slab in range(GROUP)
        ]

        def read_start(p, k, queue):
            half, slab, row = pair_reads[k]
            u = pair_units(p)[half]
            pltpu.make_async_copy(
                window(x_hbm, u, slab, 1, row, READ_SEG),
                xb.at[slot(u, n_x), pl.ds(slab, 1), pl.ds(row, READ_SEG)],
                rsem.at[p % READ_AHEAD],
            ).start(priority=queue)

        def read_wait(p):
            for u in pair_units(p):
                pltpu.make_async_copy(
                    window(x_hbm, u, 0, GROUP, 0, UNIT), xb.at[slot(u, n_x)], rsem.at[p % READ_AHEAD]
                ).wait()

        def write_wait(u):
            pltpu.make_async_copy(
                yb.at[slot(u, n_y)], window(o_hbm, u, 0, GROUP, 0, UNIT), wsem.at[u % WRITE_LAG]
            ).wait()

        def write_start(u):
            pl.when(u >= WRITE_LAG)(lambda: write_wait(u - WRITE_LAG))
            for row in range(0, UNIT, WRITE_SEG):
                pltpu.make_async_copy(
                    yb.at[slot(u, n_y), :, pl.ds(row, WRITE_SEG)],
                    window(o_hbm, u, 0, GROUP, row, WRITE_SEG),
                    wsem.at[u % WRITE_LAG],
                ).start()

        def compute(u, slab, n):
            xv = xb[slot(u, n_x), pl.ds(slab, n)].reshape(n * UNIT, C)
            acc = jnp.dot(xv, w_v[...], preferred_element_type=jnp.float32)
            acc = acc + b_v[...].astype(jnp.float32).reshape(1, D)
            yb[slot(u, n_y), pl.ds(slab, n)] = acc.astype(yb.dtype).reshape(n, UNIT, D)

        def queue_of(k):
            return READ_QUEUES[k % len(READ_QUEUES)]

        w_copy = pltpu.make_async_copy(w_hbm, w_v, csem.at[0])
        b_copy = pltpu.make_async_copy(b_hbm, b_v, csem.at[1])
        for k in range(len(pair_reads)):
            read_start(0, k, 1)
        w_copy.start()
        b_copy.start()

        def prologue(p, _):
            for k in range(len(pair_reads)):
                read_start(p, k, queue_of(k))

        lax.fori_loop(1, READ_AHEAD, prologue, None)
        w_copy.wait()
        b_copy.wait()

        def read_step(s, _):
            read_wait(s)
            per = len(pair_reads) // GROUP
            for slab in range(GROUP):
                for k in range(slab * per, (slab + 1) * per):
                    read_start(s + READ_AHEAD, k, queue_of(k))
                compute(s, slab, 1)

        lax.fori_loop(0, read_steps, read_step, None)

        def write_step(s, nxt):
            pl.when(s < n_pairs)(lambda: read_wait(s))
            write_start(nxt)
            two = nxt + 1 < s
            pl.when(two)(lambda: write_start(nxt + 1))
            compute(s, 0, GROUP)
            return nxt + 1 + two.astype(jnp.int32)

        lax.fori_loop(read_steps, n_units, write_step, jnp.int32(0))
        write_start(n_units - 1)

        def drain(u, _):
            write_wait(u)

        lax.fori_loop(n_units - WRITE_LAG, n_units, drain, None)

    out = pl.pallas_call(
        kernel_function,
        in_specs=[pl.BlockSpec(memory_space=pl.ANY)] * 3,
        out_specs=pl.BlockSpec(memory_space=pl.ANY),
        out_shape=jax.ShapeDtypeStruct((n_slabs, SLAB, D), x.dtype),
        scratch_shapes=[
            pltpu.VMEM((n_x, GROUP, UNIT, C), x.dtype),
            pltpu.VMEM((n_y, GROUP, UNIT, D), x.dtype),
            pltpu.VMEM((C, D), w.dtype),
            pltpu.VMEM((D,), b.dtype),
            pltpu.SemaphoreType.DMA((READ_AHEAD,)),
            pltpu.SemaphoreType.DMA((WRITE_LAG,)),
            pltpu.SemaphoreType.DMA((2,)),
        ],
        compiler_params=pltpu.CompilerParams(
            vmem_limit_bytes=127 * 1024 * 1024,
            disable_bounds_checks=True,
            disable_semaphore_checks=True,
        ),
    )(x.reshape(n_slabs, SLAB, C), w.reshape(C, D), b)
    return out.reshape(B, H, W, D)
```

```python
import jax
import jax.numpy as jnp
from jax import lax
import jax.experimental.pallas as pl
import jax.experimental.pallas.tpu as pltpu

SLAB = 4096
GROUP = 6
UNIT = 64
READ_SEG = 16
WRITE_SEG = 32
READ_QUEUES = (0, 1, 1, 1, 1, 1)
READ_AHEAD = 6
WRITE_LAG = 16


@jax.jit
def pallas_standalone__standard_2d_1d_3d_conv__vision_kernel(
    x: jax.Array,
    w: jax.Array,
    b: jax.Array,
):
    B, H, W, C = x.shape
    D = w.shape[-1]
    assert w.shape[0] == 1 and w.shape[1] == 1
    rows = B * H * W
    n_slabs = rows // SLAB
    per_group = SLAB // UNIT
    n_units = (n_slabs // GROUP) * per_group
    assert n_slabs * SLAB == rows and n_slabs % (2 * GROUP) == 0
    n_pairs = n_units // 2
    read_steps = n_pairs - READ_AHEAD
    n_x = n_units - read_steps + 1
    n_y = (n_units + WRITE_LAG + 2 - 2 * READ_AHEAD) // 2 + 1
    assert 2 * n_x >= n_units and 2 * n_y >= n_units

    def kernel_function(x_hbm, w_hbm, b_hbm, o_hbm, xb, yb, w_v, b_v, rsem, wsem, csem):
        def slot(u, n):
            return jnp.where(u >= n, u - n, u)

        def window(ref, u, slab, n, row, n_rows):
            off = pl.multiple_of((u % per_group) * UNIT + row, 16)
            return ref.at[pl.ds((u // per_group) * GROUP + slab, n), pl.ds(off, n_rows)]

        def pair_units(p):
            u = (p // per_group) * (2 * per_group) + p % per_group
            return u, u + per_group

        pair_reads = [
            (half, slab, row)
            for row in range(0, UNIT, READ_SEG)
            for half in range(2)
            for slab in range(GROUP)
        ]

        def read_start(p, k):
            half, slab, row = pair_reads[k]
            u = pair_units(p)[half]
            pltpu.make_async_copy(
                window(x_hbm, u, slab, 1, row, READ_SEG),
                xb.at[slot(u, n_x), pl.ds(slab, 1), pl.ds(row, READ_SEG)],
                rsem.at[p % READ_AHEAD],
            ).start(priority=READ_QUEUES[k % len(READ_QUEUES)])

        def read_wait(p):
            for u in pair_units(p):
                pltpu.make_async_copy(
                    window(x_hbm, u, 0, GROUP, 0, UNIT), xb.at[slot(u, n_x)], rsem.at[p % READ_AHEAD]
                ).wait()

        def write_wait(u):
            pltpu.make_async_copy(
                yb.at[slot(u, n_y)], window(o_hbm, u, 0, GROUP, 0, UNIT), wsem.at[u % WRITE_LAG]
            ).wait()

        def write_start(u):
            pl.when(u >= WRITE_LAG)(lambda: write_wait(u - WRITE_LAG))
            for row in range(0, UNIT, WRITE_SEG):
                pltpu.make_async_copy(
                    yb.at[slot(u, n_y), :, pl.ds(row, WRITE_SEG)],
                    window(o_hbm, u, 0, GROUP, row, WRITE_SEG),
                    wsem.at[u % WRITE_LAG],
                ).start()

        def compute(u, slab, n):
            xv = xb[slot(u, n_x), pl.ds(slab, n)].reshape(n * UNIT, C)
            acc = jnp.dot(xv, w_v[...], preferred_element_type=jnp.float32)
            acc = acc + b_v[...].astype(jnp.float32).reshape(1, D)
            yb[slot(u, n_y), pl.ds(slab, n)] = acc.astype(yb.dtype).reshape(n, UNIT, D)

        w_copy = pltpu.make_async_copy(w_hbm, w_v, csem.at[0])
        b_copy = pltpu.make_async_copy(b_hbm, b_v, csem.at[1])
        w_copy.start()
        b_copy.start()

        def prologue(p, _):
            for k in range(len(pair_reads)):
                read_start(p, k)

        lax.fori_loop(0, READ_AHEAD, prologue, None)
        w_copy.wait()
        b_copy.wait()

        def read_step(s, _):
            read_wait(s)
            per = len(pair_reads) // GROUP
            for slab in range(GROUP):
                for k in range(slab * per, (slab + 1) * per):
                    read_start(s + READ_AHEAD, k)
                compute(s, slab, 1)

        lax.fori_loop(0, read_steps, read_step, None)

        def write_step(s, nxt):
            pl.when(s < n_pairs)(lambda: read_wait(s))
            write_start(nxt)
            two = nxt + 1 < s
            pl.when(two)(lambda: write_start(nxt + 1))
            compute(s, 0, GROUP)
            return nxt + 1 + two.astype(jnp.int32)

        lax.fori_loop(read_steps, n_units, write_step, jnp.int32(0))
        write_start(n_units - 1)

        def drain(u, _):
            write_wait(u)

        lax.fori_loop(n_units - WRITE_LAG, n_units, drain, None)

    out = pl.pallas_call(
        kernel_function,
        in_specs=[pl.BlockSpec(memory_space=pl.ANY)] * 3,
        out_specs=pl.BlockSpec(memory_space=pl.ANY),
        out_shape=jax.ShapeDtypeStruct((n_slabs, SLAB, D), x.dtype),
        scratch_shapes=[
            pltpu.VMEM((n_x, GROUP, UNIT, C), x.dtype),
            pltpu.VMEM((n_y, GROUP, UNIT, D), x.dtype),
            pltpu.VMEM((C, D), w.dtype),
            pltpu.VMEM((D,), b.dtype),
            pltpu.SemaphoreType.DMA((READ_AHEAD,)),
            pltpu.SemaphoreType.DMA((WRITE_LAG,)),
            pltpu.SemaphoreType.DMA((2,)),
        ],
        compiler_params=pltpu.CompilerParams(
            vmem_limit_bytes=127 * 1024 * 1024,
            disable_bounds_checks=True,
            disable_semaphore_checks=True,
        ),
    )(x.reshape(n_slabs, SLAB, C), w.reshape(C, D), b)
    return out.reshape(B, H, W, D)
```

```python
import jax
import jax.numpy as jnp
from jax import lax
import jax.experimental.pallas as pl
import jax.experimental.pallas.tpu as pltpu

SLAB = 4096
GROUP = 6
UNIT = 64
READ_SEG = 16
WRITE_SEG = 32
READ_QUEUES = (0, 1, 1, 1, 1, 1)
READ_AHEAD = 6
WRITE_LAG = 16


@jax.jit
def pallas_standalone__standard_2d_1d_3d_conv__vision_kernel(
    x: jax.Array,
    w: jax.Array,
    b: jax.Array,
):
    B, H, W, C = x.shape
    D = w.shape[-1]
    assert w.shape[0] == 1 and w.shape[1] == 1
    rows = B * H * W
    n_slabs = rows // SLAB
    per_group = SLAB // UNIT
    n_units = (n_slabs // GROUP) * per_group
    assert n_slabs * SLAB == rows and n_slabs % (2 * GROUP) == 0
    n_pairs = n_units // 2
    read_steps = n_pairs - READ_AHEAD
    n_x = n_units - read_steps + 1
    n_y = (n_units + WRITE_LAG + 2 - 2 * READ_AHEAD) // 2 + 1
    assert 2 * n_x >= n_units and 2 * n_y >= n_units

    def kernel_function(x_hbm, w_hbm, b_hbm, o_hbm, xb, yb, w_v, b_v, rsem, wsem, csem):
        def slot(u, n):
            return jnp.where(u >= n, u - n, u)

        def window(ref, u, slab, n, row, n_rows):
            off = pl.multiple_of((u % per_group) * UNIT + row, 16)
            return ref.at[pl.ds((u // per_group) * GROUP + slab, n), pl.ds(off, n_rows)]

        def pair_units(p):
            u = (p // per_group) * (2 * per_group) + p % per_group
            return u, u + per_group

        pair_reads = [
            (*divmod(j, GROUP), row)
            for row in range(0, UNIT, READ_SEG)
            for j in (*range(0, 2 * GROUP, 2), *range(1, 2 * GROUP, 2))
        ]

        def read_start(p, k):
            half, slab, row = pair_reads[k]
            u = pair_units(p)[half]
            pltpu.make_async_copy(
                window(x_hbm, u, slab, 1, row, READ_SEG),
                xb.at[slot(u, n_x), pl.ds(slab, 1), pl.ds(row, READ_SEG)],
                rsem.at[p % READ_AHEAD],
            ).start(priority=READ_QUEUES[k % len(READ_QUEUES)])

        def read_wait(p):
            for u in pair_units(p):
                pltpu.make_async_copy(
                    window(x_hbm, u, 0, GROUP, 0, UNIT), xb.at[slot(u, n_x)], rsem.at[p % READ_AHEAD]
                ).wait()

        def write_wait(u):
            pltpu.make_async_copy(
                yb.at[slot(u, n_y)], window(o_hbm, u, 0, GROUP, 0, UNIT), wsem.at[u % WRITE_LAG]
            ).wait()

        def write_start(u):
            pl.when(u >= WRITE_LAG)(lambda: write_wait(u - WRITE_LAG))
            for row in range(0, UNIT, WRITE_SEG):
                pltpu.make_async_copy(
                    yb.at[slot(u, n_y), :, pl.ds(row, WRITE_SEG)],
                    window(o_hbm, u, 0, GROUP, row, WRITE_SEG),
                    wsem.at[u % WRITE_LAG],
                ).start()

        def compute(u, slab, n):
            xv = xb[slot(u, n_x), pl.ds(slab, n)].reshape(n * UNIT, C)
            acc = jnp.dot(xv, w_v[...], preferred_element_type=jnp.float32)
            acc = acc + b_v[...].astype(jnp.float32).reshape(1, D)
            yb[slot(u, n_y), pl.ds(slab, n)] = acc.astype(yb.dtype).reshape(n, UNIT, D)

        w_copy = pltpu.make_async_copy(w_hbm, w_v, csem.at[0])
        b_copy = pltpu.make_async_copy(b_hbm, b_v, csem.at[1])
        w_copy.start()
        b_copy.start()

        def prologue(p, _):
            for k in range(len(pair_reads)):
                read_start(p, k)

        lax.fori_loop(0, READ_AHEAD, prologue, None)
        w_copy.wait()
        b_copy.wait()

        def read_step(s, _):
            read_wait(s)
            per = len(pair_reads) // GROUP
            for slab in range(GROUP):
                for k in range(slab * per, (slab + 1) * per):
                    read_start(s + READ_AHEAD, k)
                compute(s, slab, 1)

        lax.fori_loop(0, read_steps, read_step, None)

        def write_step(s, nxt):
            pl.when(s < n_pairs)(lambda: read_wait(s))
            write_start(nxt)
            two = nxt + 1 < s
            pl.when(two)(lambda: write_start(nxt + 1))
            compute(s, 0, GROUP)
            return nxt + 1 + two.astype(jnp.int32)

        lax.fori_loop(read_steps, n_units, write_step, jnp.int32(0))
        write_start(n_units - 1)

        def drain(u, _):
            write_wait(u)

        lax.fori_loop(n_units - WRITE_LAG, n_units, drain, None)

    out = pl.pallas_call(
        kernel_function,
        in_specs=[pl.BlockSpec(memory_space=pl.ANY)] * 3,
        out_specs=pl.BlockSpec(memory_space=pl.ANY),
        out_shape=jax.ShapeDtypeStruct((n_slabs, SLAB, D), x.dtype),
        scratch_shapes=[
            pltpu.VMEM((n_x, GROUP, UNIT, C), x.dtype),
            pltpu.VMEM((n_y, GROUP, UNIT, D), x.dtype),
            pltpu.VMEM((C, D), w.dtype),
            pltpu.VMEM((D,), b.dtype),
            pltpu.SemaphoreType.DMA((READ_AHEAD,)),
            pltpu.SemaphoreType.DMA((WRITE_LAG,)),
            pltpu.SemaphoreType.DMA((2,)),
        ],
        compiler_params=pltpu.CompilerParams(
            vmem_limit_bytes=120 * 1024 * 1024,
            disable_bounds_checks=True,
            disable_semaphore_checks=True,
        ),
    )(x.reshape(n_slabs, SLAB, C), w.reshape(C, D), b)
    return out.reshape(B, H, W, D)
```

```python
import jax
import jax.numpy as jnp
from jax import lax
import jax.experimental.pallas as pl
import jax.experimental.pallas.tpu as pltpu

SLAB = 4096
GROUP = 6
UNIT = 64
READ_SEG = 16
WRITE_SEG = 32
READ_QUEUES = (0, 1, 1, 1, 1, 1)
READ_AHEAD = 6
WRITE_LAG = 16


@jax.jit
def pallas_standalone__standard_2d_1d_3d_conv__vision_kernel(
    x: jax.Array,
    w: jax.Array,
    b: jax.Array,
):
    B, H, W, C = x.shape
    D = w.shape[-1]
    assert w.shape[0] == 1 and w.shape[1] == 1
    rows = B * H * W
    n_slabs = rows // SLAB
    per_group = SLAB // UNIT
    n_units = (n_slabs // GROUP) * per_group
    assert n_slabs * SLAB == rows and n_slabs % (2 * GROUP) == 0
    n_pairs = n_units // 2
    read_steps = n_pairs - READ_AHEAD
    n_x = n_units - read_steps + 1
    n_y = (n_units + WRITE_LAG + 2 - 2 * READ_AHEAD) // 2 + 1
    assert 2 * n_x >= n_units and 2 * n_y >= n_units

    def kernel_function(x_hbm, w_hbm, b_hbm, o_hbm, xb, yb, w_v, b_v, rsem, wsem, csem):
        def slot(u, n):
            return jnp.where(u >= n, u - n, u)

        def window(ref, u, slab, n, row, n_rows):
            off = pl.multiple_of((u % per_group) * UNIT + row, 16)
            return ref.at[pl.ds((u // per_group) * GROUP + slab, n), pl.ds(off, n_rows)]

        def pair_units(p):
            u = (p // per_group) * (2 * per_group) + p % per_group
            return u, u + per_group

        pair_reads = [
            (*divmod(j, GROUP), row)
            for row in range(0, UNIT, READ_SEG)
            for j in (*range(0, 2 * GROUP, 2), *range(1, 2 * GROUP, 2))
        ]

        def read_start(p, k):
            half, slab, row = pair_reads[k]
            u = pair_units(p)[half]
            pltpu.make_async_copy(
                window(x_hbm, u, slab, 1, row, READ_SEG),
                xb.at[slot(u, n_x), pl.ds(slab, 1), pl.ds(row, READ_SEG)],
                rsem.at[half, p % READ_AHEAD],
            ).start(priority=READ_QUEUES[k % len(READ_QUEUES)])

        def read_wait(p):
            for half, u in enumerate(pair_units(p)):
                pltpu.make_async_copy(
                    window(x_hbm, u, 0, GROUP, 0, UNIT),
                    xb.at[slot(u, n_x)],
                    rsem.at[half, p % READ_AHEAD],
                ).wait()

        def write_wait(u):
            pltpu.make_async_copy(
                yb.at[slot(u, n_y)], window(o_hbm, u, 0, GROUP, 0, UNIT), wsem.at[u % WRITE_LAG]
            ).wait()

        def write_start(u):
            pl.when(u >= WRITE_LAG)(lambda: write_wait(u - WRITE_LAG))
            for row in range(0, UNIT, WRITE_SEG):
                pltpu.make_async_copy(
                    yb.at[slot(u, n_y), :, pl.ds(row, WRITE_SEG)],
                    window(o_hbm, u, 0, GROUP, row, WRITE_SEG),
                    wsem.at[u % WRITE_LAG],
                ).start()

        def compute(u, slab, n):
            xv = xb[slot(u, n_x), pl.ds(slab, n)].reshape(n * UNIT, C)
            acc = jnp.dot(xv, w_v[...], preferred_element_type=jnp.float32)
            acc = acc + b_v[...].astype(jnp.float32).reshape(1, D)
            yb[slot(u, n_y), pl.ds(slab, n)] = acc.astype(yb.dtype).reshape(n, UNIT, D)

        w_copy = pltpu.make_async_copy(w_hbm, w_v, csem.at[0])
        b_copy = pltpu.make_async_copy(b_hbm, b_v, csem.at[1])
        w_copy.start()
        b_copy.start()

        def prologue(p, _):
            for k in range(len(pair_reads)):
                read_start(p, k)

        lax.fori_loop(0, READ_AHEAD, prologue, None)
        w_copy.wait()
        b_copy.wait()

        def read_step(s, _):
            read_wait(s)
            per = len(pair_reads) // GROUP
            for slab in range(GROUP):
                for k in range(slab * per, (slab + 1) * per):
                    read_start(s + READ_AHEAD, k)
                compute(s, slab, 1)

        lax.fori_loop(0, read_steps, read_step, None)

        def write_step(s, nxt):
            pl.when(s < n_pairs)(lambda: read_wait(s))
            write_start(nxt)
            two = nxt + 1 < s
            pl.when(two)(lambda: write_start(nxt + 1))
            compute(s, 0, GROUP)
            return nxt + 1 + two.astype(jnp.int32)

        lax.fori_loop(read_steps, n_units, write_step, jnp.int32(0))
        write_start(n_units - 1)

        def drain(u, _):
            write_wait(u)

        lax.fori_loop(n_units - WRITE_LAG, n_units, drain, None)

    out = pl.pallas_call(
        kernel_function,
        in_specs=[pl.BlockSpec(memory_space=pl.ANY)] * 3,
        out_specs=pl.BlockSpec(memory_space=pl.ANY),
        out_shape=jax.ShapeDtypeStruct((n_slabs, SLAB, D), x.dtype),
        scratch_shapes=[
            pltpu.VMEM((n_x, GROUP, UNIT, C), x.dtype),
            pltpu.VMEM((n_y, GROUP, UNIT, D), x.dtype),
            pltpu.VMEM((C, D), w.dtype),
            pltpu.VMEM((D,), b.dtype),
            pltpu.SemaphoreType.DMA((2, READ_AHEAD)),
            pltpu.SemaphoreType.DMA((WRITE_LAG,)),
            pltpu.SemaphoreType.DMA((2,)),
        ],
        compiler_params=pltpu.CompilerParams(
            vmem_limit_bytes=120 * 1024 * 1024,
            disable_bounds_checks=True,
            disable_semaphore_checks=True,
        ),
    )(x.reshape(n_slabs, SLAB, C), w.reshape(C, D), b)
    return out.reshape(B, H, W, D)
```
